```python
import os as _os
_os.environ.setdefault("JAX_PLATFORMS", "cpu")
import jax
import jax.numpy as jnp

def _softmax(x, axis=-1):
    return jax.nn.softmax(x, axis=axis)
def _gelu(x):
    return jax.nn.gelu(x, approximate=True)
def _silu(x):
    return jax.nn.silu(x)
def _sigmoid(x):
    return jax.nn.sigmoid(x)
def _layernorm(x, axis=-1, eps=1e-5):
    m = jnp.mean(x, axis=axis, keepdims=True)
    v = jnp.var(x, axis=axis, keepdims=True)
    return (x - m) / jnp.sqrt(v + eps)
def _scatter_add(tgt, idx, src, axis=0):
    return tgt.at[idx].add(src)
def _segment_sum(src, seg, n):
    return jax.ops.segment_sum(src, seg, n)
class _Rng:
    def __init__(self, key):
        self._k = key
    def _next(self):
        self._k, sub = jax.random.split(self._k)
        return sub
    def normal(self, shape):
        return jax.random.normal(self._next(), shape, dtype=jnp.bfloat16)
    def randint(self, lo, hi, shape):
        return jax.random.randint(self._next(), shape, lo, hi, dtype=jnp.int32)
    def uniform(self, shape, lo=0.0, hi=1.0):
        return jax.random.uniform(self._next(), shape, jnp.bfloat16, lo, hi)
    def permutation(self, n):
        return jax.random.permutation(self._next(), n)


kernel_name = 'standalone__mha_block_cached__near_ridge'

def setup_inputs():
    _rng = _Rng(jax.random.key(int.from_bytes(__import__("os").urandom(4), "little")))
    _w = (lambda a: (lambda t: t.astype(jnp.bfloat16) if jnp.issubdtype(t.dtype, jnp.floating) else t)(jnp.asarray(a)))
    B, Sq, D = 8, 96, 576
    H, Sk, Dh = 32, 96, 128
    return {
        "x": _w((lambda *s: _rng.normal(s) * 0.8)(B, Sq, D)),
        "k_cache": _w((lambda *s: _rng.normal(s) * 0.8)(B, H, Sk, Dh)),
        "v_cache": _w((lambda *s: _rng.normal(s) * 0.05)(B, H, Sk, Dh)),
        "wq": _w((lambda *s: _rng.normal(s) * 0.8)(D, H * Dh) * (D ** -0.5)),
        "wo": _w((lambda *s: _rng.normal(s) * 0.05)(H * Dh, D) * ((H * Dh) ** -0.5)),
    }

def reference(x, k_cache, v_cache, wq, wo):
    B, Sq, D = x.shape
    H, Dh = 32, 128
    q = (lambda x, *d: x.transpose(*d))((x @ wq).reshape(B, Sq, H, Dh), 0, 2, 1, 3)
    scores = jnp.einsum("bhqd,bhkd->bhqk", q, k_cache) * (Dh ** -0.5)
    p = _softmax(scores, axis=-1)
    o = jnp.einsum("bhqk,bhkd->bhqd", p, v_cache)
    return (lambda x, *d: x.transpose(*d))(o, 0, 2, 1, 3).reshape(B, Sq, H * Dh) @ wo
```

```python
import jax, jax.numpy as jnp
from jax import lax
import jax.experimental.pallas as pl
import jax.experimental.pallas.tpu as pltpu

B, SQ, D, H, SK, DH = 8, 96, 576, 32, 96, 128
M = B * SQ
NT = (((1,), (1,)), ((), ()))

def _make(G=4, rcp=2, order='Sqop', order_q='Sqp', order_o='Sop', LAG=5, PAD=0, RC=128, SL=(4,4,8,4,4,8), pre=False, U=1, U2=1, XS=(0, 128, 256, 384, 576),):
    NG = H // G
    NR = M // 128
    def kern(x_hbm, k_hbm, v_hbm, wq_hbm, wot_hbm, o_hbm,
             x_v, k_v, v_v, wq_v, wot_v, q_v, a_v, acc_v, y_v, q32, sem_x, sem_g, sem_o):
        def cs(g):
            return pl.ds(pl.multiple_of(g * (G * DH), G * DH), G * DH)
        def cq(g):
            return pltpu.make_async_copy(wq_hbm.at[:, cs(g)], wq_v.at[g], sem_g.at[0, g])
        def ck(g):
            hs = pl.ds(g * G, G)
            return pltpu.make_async_copy(k_hbm.at[:, hs], k_v.at[:, hs], sem_g.at[1, g])
        def cv(g):
            hs = pl.ds(g * G, G)
            return pltpu.make_async_copy(v_hbm.at[:, hs], v_v.at[:, hs], sem_g.at[2, g])
        def cw(g):
            return pltpu.make_async_copy(wot_hbm.at[:, cs(g)], wot_v.at[g], sem_g.at[3, g])
        def co(r):
            rs = pl.ds(r * 128, 128)
            return pltpu.make_async_copy(y_v.at[rs], o_hbm.at[rs], sem_o.at[r])

        def qproj(g, r0, r1):
            q = jnp.dot(x_v[r0:r1, :], wq_v[g], preferred_element_type=jnp.float32)
            q_v[g, r0:r1, :] = q.astype(jnp.bfloat16)

        cst = (DH ** -0.5) * 1.4426950408889634
        def att_s(g, b, h):
            qb = q_v[g, b*SQ:(b+1)*SQ, h*DH:(h+1)*DH]
            s = lax.dot_general(qb, k_v[b, g*G + h], NT, preferred_element_type=jnp.float32)
            m = jnp.max(s, axis=-1, keepdims=True)
            e = jnp.exp2((s - m) * cst)
            l = jnp.sum(e, axis=-1, keepdims=True)
            r = pl.reciprocal(l, approx=True)
            if rcp == 2:
                r = r * (2.0 - l * r)
            if pre: return (e * r).astype(jnp.bfloat16), None
            return e.astype(jnp.bfloat16), r
        def att_p(g, b, h, e, r):
            o = jnp.dot(e, v_v[b, g*G + h], preferred_element_type=jnp.float32)
            if r is not None: o = o * r
            a_v[0, b*SQ:(b+1)*SQ, h*DH:(h+1)*DH] = o.astype(jnp.bfloat16)

        def outp(g, r, last=False):
            a = a_v[0, r*128:(r+1)*128, :]
            yt = acc_v[r] + lax.dot_general(wot_v[g], a, NT, preferred_element_type=jnp.float32)
            if last:
                y_v[r*128:(r+1)*128, :] = yt.T.astype(jnp.bfloat16)
                co(r).start()
            else:
                acc_v[r] = yt

        pairs = [(b, h) for b in range(B) for h in range(G)]
        def stage(g, doq, doa, doo):
            od = order if (doq and doo) else (order_q if doq else order_o)
            cuts = [sum(SL[:i]) for i in range(7)]
            st = {}
            if 'S' in od:
                for p in pairs[cuts[0]:cuts[1]]: st[p] = att_s(g, *p)
            for r in range(6):
                for c in od:
                    if c == 'q': qproj(g + 2, r*128, (r+1)*128)
                    if c == 'o': outp(g - 1, r)
                    if c in 'sS':
                        rr = r if c == 's' else r + 1
                        if rr < 6:
                            for p in pairs[cuts[rr]:cuts[rr+1]]: st[p] = att_s(g, *p)
                    if c == 'p':
                        for p in pairs[cuts[r]:cuts[r+1]]: att_p(g, *p, *st[p])

        KS = XS
        nk = len(KS) - 1
        def cxk(i):
            return pltpu.make_async_copy(x_hbm.at[:, KS[i]:KS[i+1]], x_v.at[:, KS[i]:KS[i+1]], sem_x.at[i])
        def cqk(i):
            return pltpu.make_async_copy(wq_hbm.at[KS[i]:KS[i+1], 0:G*DH], wq_v.at[0, KS[i]:KS[i+1], :], sem_x.at[8 + i])
        for i in range(nk):
            cqk(i).start(); cxk(i).start()
        cq(1).start()
        for i in range(nk):
            cqk(i).wait(); cxk(i).wait()
            if i == 0:
                ck(0).start(); cv(0).start(); cq(2).start()
            rc = RC if i == nk - 1 else M
            for r0 in range(0, M, rc):
                p = jnp.dot(x_v[r0:r0+rc, KS[i]:KS[i+1]], wq_v[0, KS[i]:KS[i+1], :], preferred_element_type=jnp.float32)
                if i > 0: p = p + q32[r0:r0+rc, :]
                if i < nk - 1: q32[r0:r0+rc, :] = p
                else: q_v[0, r0:r0+rc, :] = p.astype(jnp.bfloat16)
        acc_v[...] = jnp.zeros_like(acc_v)
        cq(1).wait()
        qproj(1, 0, M)
        cq(2).wait(); ck(0).wait(); cv(0).wait()
        cq(3).start(); ck(1).start(); cv(1).start(); cw(0).start()
        stage(0, True, True, False)

        def body(g, _):
            cq(g + 2).wait(); ck(g).wait(); cv(g).wait(); cw(g - 1).wait()
            @pl.when(g + 3 < NG)
            def _():
                cq(g + 3).start()
            ck(g + 1).start(); cv(g + 1).start(); cw(g).start()
            stage(g, True, True, True)
            return 0
        lax.fori_loop(1, NG - 2, body, 0, unroll=U)
        def body2(g, _):
            ck(g).wait(); cv(g).wait(); cw(g - 1).wait()
            @pl.when(g + 1 < NG)
            def _():
                ck(g + 1).start(); cv(g + 1).start()
            cw(g).start()
            stage(g, False, True, True)
            return 0
        lax.fori_loop(NG - 2, NG, body2, 0, unroll=U2)
        g = NG - 1
        cw(g).wait()
        for r in range(NR):
            if r == LAG: co(0).wait()
            outp(g, r, last=True)
        for r in range(1 if LAG < NR else 0, NR):
            co(r).wait()

    @jax.jit
    def fn(x, k_cache, v_cache, wq, wo):
        hbm = pl.BlockSpec(memory_space=pltpu.HBM)
        out = pl.pallas_call(
            kern,
            in_specs=[hbm] * 5,
            out_specs=hbm,
            out_shape=jax.ShapeDtypeStruct((M, D), jnp.bfloat16),
            scratch_shapes=[
                pltpu.VMEM((M, D), jnp.bfloat16),
                pltpu.VMEM((B, H, SK, DH), jnp.bfloat16),
                pltpu.VMEM((B, H, SK, DH), jnp.bfloat16),
                pltpu.VMEM((NG, D, G * DH), jnp.bfloat16),
                pltpu.VMEM((NG, D, G * DH), jnp.bfloat16),
                pltpu.VMEM((NG, M, G * DH), jnp.bfloat16),
                pltpu.VMEM((1, M, G * DH), jnp.bfloat16),
                pltpu.VMEM((NR, D, 128), jnp.float32),
                pltpu.VMEM((M, D), jnp.bfloat16),
                pltpu.VMEM((M + PAD, G*DH), jnp.float32),
                pltpu.SemaphoreType.DMA((16,)),
                pltpu.SemaphoreType.DMA((4, NG)),
                pltpu.SemaphoreType.DMA((NR,)),
            ],
            compiler_params=pltpu.CompilerParams(vmem_limit_bytes=100*1024*1024),
        )(x.reshape(M, D), k_cache, v_cache, wq, wo.T)
        return out.reshape(B, SQ, D)
    return fn


_kernel = _make()


@jax.jit
def pallas_standalone__mha_block_cached__near_ridge_kernel(x, k_cache, v_cache, wq, wo):
    return _kernel(x, k_cache, v_cache, wq, wo)
```
